```python
import jax
import jax.numpy as jnp

def _softmax(x, axis=-1):
    return jax.nn.softmax(x, axis=axis)
def _gelu(x):
    return jax.nn.gelu(x, approximate=True)
def _silu(x):
    return jax.nn.silu(x)
def _sigmoid(x):
    return jax.nn.sigmoid(x)
def _layernorm(x, axis=-1, eps=1e-5):
    m = jnp.mean(x, axis=axis, keepdims=True)
    v = jnp.var(x, axis=axis, keepdims=True)
    return (x - m) / jnp.sqrt(v + eps)
def _scatter_add(tgt, idx, src, axis=0):
    return tgt.at[idx].add(src)
def _segment_sum(src, seg, n):
    return jax.ops.segment_sum(src, seg, n)
class _Rng:
    def __init__(self, key):
        self._k = key
    def _next(self):
        self._k, sub = jax.random.split(self._k)
        return sub
    def normal(self, shape):
        return jax.random.normal(self._next(), shape, dtype=jnp.bfloat16)
    def randint(self, lo, hi, shape):
        return jax.random.randint(self._next(), shape, lo, hi, dtype=jnp.int32)
    def uniform(self, shape, lo=0.0, hi=1.0):
        return jax.random.uniform(self._next(), shape, jnp.bfloat16, lo, hi)
    def permutation(self, n):
        return jax.random.permutation(self._next(), n)


kernel_name = 'interleave_layers__sliding_local_dilated__glu_gated_bilinear__prompt'

def setup_inputs():
    _rng = _Rng(jax.random.key(int.from_bytes(__import__("os").urandom(4), "little")))
    _w = (lambda a: (lambda t: t.astype(jnp.bfloat16) if jnp.issubdtype(t.dtype, jnp.floating) else t)(jnp.asarray(a)))
    def _A_setup():
        B, S, D = 1, 2048, 576
        return {
            "x": _w((lambda *s: _rng.normal(s) * 0.05)(B, S, D)),
            "wqkv": _w((lambda *s: _rng.normal(s) * 0.05)(D, 3 * D)),
            "wo": _w((lambda *s: _rng.normal(s) * 0.05)(D, D)),
        }
    _A_in = _A_setup()

    def _B_setup():
        B, S, D, F = 1, 2048, 576, 4608
        return {
            "x": _w((lambda *s: _rng.normal(s) * 0.05)(B, S, D)),
            "w_gate": _w((lambda *s: _rng.normal(s) * 0.05)(D, F) * (D ** -0.5)),
            "w_up": _w((lambda *s: _rng.normal(s) * 0.05)(D, F) * (D ** -0.5)),
            "w_down": _w((lambda *s: _rng.normal(s) * 0.05)(F, D) * (F ** -0.5)),
        }
    _B_in = _B_setup()

    return {
        "A_x": _A_in["x"],
        "A_wqkv": _A_in["wqkv"],
        "A_wo": _A_in["wo"],
        "B_x": _B_in["x"],
        "B_w_gate": _B_in["w_gate"],
        "B_w_up": _B_in["w_up"],
        "B_w_down": _B_in["w_down"],
    }

def reference(A_x, A_wqkv, A_wo, B_x, B_w_gate, B_w_up, B_w_down):
    def _A_ref(x, wqkv, wo):
        B, S, D = x.shape
        H = 32; Dh = D // H
        W, dil = 8, 2
        qkv = (lambda x, *d: x.transpose(*d))((x @ wqkv).reshape(B, S, 3, H, Dh), 2, 0, 3, 1, 4)
        q, k, v = qkv[0], qkv[1], qkv[2]
        scale = Dh ** -0.5
        pos = jnp.arange(S)
        off = jnp.arange(W) * dil
        idx = pos[:, None] - off[None, :]
        mask = idx >= 0
        idx_c = jnp.where(mask, idx, 0).reshape(-1)
        kg = k[:, :, idx_c, :].reshape(B, H, S, W, Dh)
        vg = v[:, :, idx_c, :].reshape(B, H, S, W, Dh)
        logits = jnp.einsum("bhsd,bhswd->bhsw", q, kg) * scale
        logits = jnp.where(mask[None, None, :, :], logits, -1e9)
        attn = _softmax(logits, axis=-1)
        o = jnp.einsum("bhsw,bhswd->bhsd", attn, vg)
        return (lambda x, *d: x.transpose(*d))(o, 0, 2, 1, 3).reshape(B, S, D) @ wo

    def _B_ref(x, w_gate, w_up, w_down):
        g = jnp.einsum("bsd,df->bsf", x, w_gate)
        u = jnp.einsum("bsd,df->bsf", x, w_up)
        h = g * u
        return jnp.einsum("bsf,fd->bsd", h, w_down)

    x = A_x
    x = x + _A_ref(_layernorm(x, axis=-1), A_wqkv, A_wo)
    x = x + _B_ref(_layernorm(x, axis=-1), B_w_gate, B_w_up, B_w_down)
    x = x + _A_ref(_layernorm(x, axis=-1), A_wqkv, A_wo)
    x = x + _B_ref(_layernorm(x, axis=-1), B_w_gate, B_w_up, B_w_down)
    return x
```

```python
import math

import jax
import jax.numpy as jnp
import jax.experimental.pallas as pl
import jax.experimental.pallas.tpu as pltpu

H, W, DIL = 32, 8, 2
BF, F32 = jnp.bfloat16, jnp.float32
TN = (((0,), (0,)), ((), ()))
TA = 256
TF = 512
FC = 512


def _dot(a, b):
    return jnp.dot(a, b, preferred_element_type=F32)


def _ln(x):
    m = jnp.mean(x, axis=0, keepdims=True)
    c = x - m
    v = jnp.mean(c * c, axis=0, keepdims=True)
    return (c * jax.lax.rsqrt(v + 1e-5)).astype(BF)


def _kernel(x_hbm, wqkv_hbm, wo_hbm, wg_hbm, wu_hbm, wd_hbm, o_hbm,
            xin, wqkv_v, wo_v, wg, wu, wd, wq_p, wo_p, tmp, xs, xn, sems):
    D, S = xs.shape
    DH = D // H
    F = wd.shape[1]
    loads = [pltpu.make_async_copy(s, d, sems.at[i]) for i, (s, d) in enumerate(
        [(wqkv_hbm, wqkv_v), (x_hbm, xin), (wo_hbm, wo_v),
         (wg_hbm, wg), (wu_hbm, wu), (wd_hbm, wd)])]
    for c in loads:
        c.start()

    def perm_rows(val):
        nt = -(-D // 128)
        val = jnp.concatenate([val, jnp.zeros((D, nt * 128 - D), F32)], axis=1)
        for j in range(nt):
            tmp[j * D:(j + 1) * D, :] = val[:, j * 128:(j + 1) * 128]
        return jnp.concatenate([
            jnp.concatenate([tmp[pl.ds(j * D + d, H, stride=DH), :]
                             for d in range(DH)], axis=0)
            for j in range(nt)], axis=1)[:, :D]

    loads[0].wait()
    for p in range(3):
        wq_p[p * D:(p + 1) * D, :] = perm_rows(
            wqkv_v[:, p * D:(p + 1) * D].astype(F32).T).astype(BF)
    loads[2].wait()
    wo_p[...] = perm_rows(wo_v[...].astype(F32)).T.astype(BF)
    loads[1].wait()
    xs[...] = xin[...].astype(F32)

    lane = jax.lax.broadcasted_iota(jnp.int32, (H, 128), 1)
    c2 = DH ** -0.5 * math.log2(math.e)

    def shifted(cur, prev, w):
        if w == 0:
            return cur
        sh = DIL * w
        if prev is not None:
            cur = jnp.where(lane >= 128 - sh, prev, cur)
        return pltpu.roll(cur, sh, 1)

    def attend(q, k, v, kp, vp):
        r = lambda a, d: None if a is None else a[d * H:(d + 1) * H]
        lg = []
        for w in range(W):
            acc = None
            for d in range(DH):
                t = r(q, d) * shifted(r(k, d), r(kp, d), w)
                acc = t if acc is None else acc + t
            acc = acc * c2
            if kp is None and w > 0:
                acc = jnp.where(lane >= DIL * w, acc, -1e9)
            lg.append(acc)
        m = lg[0]
        for a in lg[1:]:
            m = jnp.maximum(m, a)
        e = [jnp.exp2(a - m) for a in lg]
        inv = 1.0 / sum(e[1:], e[0])
        pr = [a * inv for a in e]
        outs = []
        for d in range(DH):
            acc = None
            for w in range(W):
                t = pr[w] * shifted(r(v, d), r(vp, d), w)
                acc = t if acc is None else acc + t
            outs.append(acc.astype(BF))
        return jnp.concatenate(outs, axis=0)

    def layer(l, _):
        kp = vp = None
        for b in range(S // TA):
            cols = slice(b * TA, (b + 1) * TA)
            x = xs[:, cols]
            qkv = _dot(wq_p[...], _ln(x))
            os = []
            for t in range(TA // 128):
                c = slice(t * 128, (t + 1) * 128)
                q, k, v = (qkv[p * D:(p + 1) * D, c] for p in range(3))
                os.append(attend(q, k, v, kp, vp))
                kp, vp = k, v
            x = x + _dot(wo_p[...], jnp.concatenate(os, axis=1))
            xs[:, cols] = x
            xn[:, cols] = _ln(x)

        @pl.when(l == 0)
        def _():
            for c in loads[3:]:
                c.wait()

        def ffn(b, _):
            cols = pl.ds(pl.multiple_of(b * TF, TF), TF)
            a = xn[:, cols]
            acc = xs[:, cols]
            for j in range(F // FC):
                c = slice(j * FC, (j + 1) * FC)
                g = jax.lax.dot_general(wg[:, c], a, TN, preferred_element_type=F32)
                u = jax.lax.dot_general(wu[:, c], a, TN, preferred_element_type=F32)
                acc = acc + _dot(wd[:, c], (g * u).astype(BF))
            xs[:, cols] = acc
            xin[:, cols] = acc.astype(BF)

            @pl.when(l == 1)
            def _():
                pltpu.make_async_copy(xin.at[:, cols], o_hbm.at[:, cols],
                                      sems.at[6 + b]).start()

        jax.lax.fori_loop(0, S // TF, ffn, None)

    jax.lax.fori_loop(0, 2, layer, None)
    for b in range(S // TF):
        cols = pl.ds(b * TF, TF)
        pltpu.make_async_copy(xin.at[:, cols], o_hbm.at[:, cols], sems.at[6 + b]).wait()


@jax.jit
def pallas_interleave_layers__sliding_local_dilated__glu_gated_bilinear__prompt_kernel(
    A_x: jax.Array,
    A_wqkv: jax.Array,
    A_wo: jax.Array,
    B_x: jax.Array,
    B_w_gate: jax.Array,
    B_w_up: jax.Array,
    B_w_down: jax.Array,
):
    _, S, D = A_x.shape
    F = B_w_gate.shape[1]
    V = pltpu.VMEM
    out = pl.pallas_call(
        _kernel,
        in_specs=[pl.BlockSpec(memory_space=pl.ANY)] * 6,
        out_specs=pl.BlockSpec(memory_space=pl.ANY),
        out_shape=jax.ShapeDtypeStruct((D, S), A_x.dtype),
        scratch_shapes=[
            V((D, S), BF), V((D, 3 * D), BF), V((D, D), BF),
            V((D, F), BF), V((D, F), BF), V((D, F), BF),
            V((3 * D, D), BF), V((D, D), BF), V((-(-D // 128) * D, 128), F32),
            V((D, S), F32), V((D, S), BF),
            pltpu.SemaphoreType.DMA((6 + S // TF,)),
        ],
        compiler_params=pltpu.CompilerParams(vmem_limit_bytes=100 << 20),
    )(A_x[0].T, A_wqkv, A_wo, B_w_gate, B_w_up, B_w_down.T)
    return out.T[None]
```

```python
import math

import jax
import jax.numpy as jnp
import jax.experimental.pallas as pl
import jax.experimental.pallas.tpu as pltpu

H, W, DIL = 32, 8, 2
BF, F32 = jnp.bfloat16, jnp.float32
TN = (((0,), (0,)), ((), ()))
TB = 256
LA = 3
KVT = F32
FC = 512


def _dot(a, b):
    return jnp.dot(a, b, preferred_element_type=F32)


def _ln(x):
    m = jnp.mean(x, axis=0, keepdims=True)
    c = x - m
    v = jnp.mean(c * c, axis=0, keepdims=True)
    return (c * jax.lax.rsqrt(v + 1e-5)).astype(BF)


def _kernel(x_hbm, wqkv_hbm, wo_hbm, wg_hbm, wu_hbm, wd_hbm, o_hbm,
            xin, wqkv_v, wo_v, wg, wu, wd, wq_p, wo_p, tmp, xs, xn, kv, sems):
    D, S = xs.shape
    DH = D // H
    F = wd.shape[1]
    loads = [pltpu.make_async_copy(s, d, sems.at[i]) for i, (s, d) in enumerate(
        [(wqkv_hbm, wqkv_v), (x_hbm, xin), (wo_hbm, wo_v),
         (wg_hbm, wg), (wu_hbm, wu), (wd_hbm, wd)])]
    for c in loads[:3]:
        c.start()

    def perm_rows(val):
        nt = -(-D // 128)
        val = jnp.concatenate([val, jnp.zeros((D, nt * 128 - D), F32)], axis=1)
        for j in range(nt):
            tmp[j * D:(j + 1) * D, :] = val[:, j * 128:(j + 1) * 128]
        return jnp.concatenate([
            jnp.concatenate([tmp[pl.ds(j * D + d, H, stride=DH), :]
                             for d in range(DH)], axis=0)
            for j in range(nt)], axis=1)[:, :D]

    for c in loads[:3]:
        c.wait()
    for c in loads[3:]:
        c.start()
    for p in range(3):
        wq_p[p * D:(p + 1) * D, :] = perm_rows(
            wqkv_v[:, p * D:(p + 1) * D].astype(F32).T).astype(BF)
    wo_p[...] = perm_rows(wo_v[...].astype(F32)).T.astype(BF)
    xs[...] = xin[...].astype(F32)

    lane = jax.lax.broadcasted_iota(jnp.int32, (H, 128), 1)
    c2 = DH ** -0.5 * math.log2(math.e)

    def shifted(cur, prev, w):
        if w == 0:
            return cur.astype(F32)
        sh = DIL * w
        if prev is not None:
            cur = jnp.where(lane >= 128 - sh, prev, cur)
        return pltpu.roll(cur, sh, 1).astype(F32)

    def attend(q, k, v, kp, vp, b):
        r = lambda a, d: None if a is None else a[d * H:(d + 1) * H]
        lg = []
        for w in range(W):
            acc = None
            for d in range(DH):
                t = r(q, d) * shifted(r(k, d), r(kp, d), w)
                acc = t if acc is None else acc + t
            acc = acc * c2
            if b is not None and w > 0:
                acc = jnp.where(lane + b * 128 >= DIL * w, acc, -1e9)
            lg.append(acc)
        m = lg[0]
        for a in lg[1:]:
            m = jnp.maximum(m, a)
        e = [jnp.exp2(a - m) for a in lg]
        inv = 1.0 / sum(e[1:], e[0])
        pr = [a * inv for a in e]
        outs = []
        for d in range(DH):
            acc = None
            for w in range(W):
                t = pr[w] * shifted(r(v, d), r(vp, d), w)
                acc = t if acc is None else acc + t
            outs.append(acc.astype(BF))
        return jnp.concatenate(outs, axis=0)

    nb = S // TB
    blk = lambda t: pl.ds(pl.multiple_of((t % nb) * TB, TB), TB)
    out_copy = lambda b: pltpu.make_async_copy(
        xin.at[:, blk(b)], o_hbm.at[:, blk(b)], sems.at[6 + b])

    def stage(ta, tf):
        if ta is not None:
            x = xs[:, blk(ta)]
            kp, vp = kv[0], kv[1]
        if tf is not None:
            a = xn[:, blk(tf)]
            acc = xs[:, blk(tf)]
        if ta is not None:
            qkv = _dot(wq_p[...], _ln(x))
            os = []
            for t in range(TB // 128):
                c = slice(t * 128, (t + 1) * 128)
                q, k, v = (qkv[p * D:(p + 1) * D, c] for p in range(3))
                k, v = k.astype(KVT), v.astype(KVT)
                os.append(attend(q, k, v, kp, vp, ta % nb if t == 0 else None))
                kp, vp = k, v
            kv[0] = kp
            kv[1] = vp
        if tf is not None:
            for j in range(F // FC):
                c = slice(j * FC, (j + 1) * FC)
                g = jax.lax.dot_general(wg[:, c], a, TN, preferred_element_type=F32)
                u = jax.lax.dot_general(wu[:, c], a, TN, preferred_element_type=F32)
                acc = acc + _dot(wd[:, c], (g * u).astype(BF))
        if ta is not None:
            x = x + _dot(wo_p[...], jnp.concatenate(os, axis=1))
            xs[:, blk(ta)] = x
            xn[:, blk(ta)] = _ln(x)
        if tf is not None:
            xs[:, blk(tf)] = acc
            xin[:, blk(tf)] = acc.astype(BF)

            @pl.when(tf >= nb)
            def _():
                out_copy(tf - nb).start()

    kv[...] = jnp.zeros_like(kv)
    jax.lax.fori_loop(0, LA, lambda t, _: stage(t, None), None)
    for c in loads[3:]:
        c.wait()
    jax.lax.fori_loop(0, 2 * nb - LA, lambda t, _: stage(t + LA, t), None)
    jax.lax.fori_loop(2 * nb - LA, 2 * nb, lambda t, _: stage(None, t), None)
    for b in range(nb):
        out_copy(b).wait()


@jax.jit
def pallas_interleave_layers__sliding_local_dilated__glu_gated_bilinear__prompt_kernel(
    A_x: jax.Array,
    A_wqkv: jax.Array,
    A_wo: jax.Array,
    B_x: jax.Array,
    B_w_gate: jax.Array,
    B_w_up: jax.Array,
    B_w_down: jax.Array,
):
    _, S, D = A_x.shape
    F = B_w_gate.shape[1]
    V = pltpu.VMEM
    out = pl.pallas_call(
        _kernel,
        in_specs=[pl.BlockSpec(memory_space=pl.ANY)] * 6,
        out_specs=pl.BlockSpec(memory_space=pl.ANY),
        out_shape=jax.ShapeDtypeStruct((D, S), A_x.dtype),
        scratch_shapes=[
            V((D, S), BF), V((D, 3 * D), BF), V((D, D), BF),
            V((D, F), BF), V((D, F), BF), V((D, F), BF),
            V((3 * D, D), BF), V((D, D), BF), V((-(-D // 128) * D, 128), F32),
            V((D, S), F32), V((D, S), BF), V((2, D, 128), KVT),
            pltpu.SemaphoreType.DMA((6 + S // TB,)),
        ],
        compiler_params=pltpu.CompilerParams(vmem_limit_bytes=100 << 20),
    )(A_x[0].T, A_wqkv, A_wo, B_w_gate, B_w_up, B_w_down.T)
    return out.T[None]
```

```python
import math

import jax
import jax.numpy as jnp
import jax.experimental.pallas as pl
import jax.experimental.pallas.tpu as pltpu

H, W, DIL = 32, 8, 2
BF, F32 = jnp.bfloat16, jnp.float32
TN = (((0,), (0,)), ((), ()))
TB = 256
LA = 3
KVT = F32
FC = 512


def _dot(a, b):
    return jnp.dot(a, b, preferred_element_type=F32)


def _ln(x):
    m = jnp.mean(x, axis=0, keepdims=True)
    c = x - m
    v = jnp.mean(c * c, axis=0, keepdims=True)
    return (c * jax.lax.rsqrt(v + 1e-5)).astype(BF)


def _kernel(x_hbm, wqkv_hbm, wo_hbm, wg_hbm, wu_hbm, wd_hbm, o_hbm,
            xin, wqkv_v, wo_v, wg, wu, wd, wq_p, wo_p, tmp, xs, xn, kv, sems):
    D, S = xs.shape
    DH = D // H
    F = wd.shape[1]
    loads = [pltpu.make_async_copy(s, d, sems.at[i]) for i, (s, d) in enumerate(
        [(wqkv_hbm, wqkv_v), (x_hbm, xin), (wo_hbm, wo_v),
         (wg_hbm, wg), (wu_hbm, wu), (wd_hbm, wd)])]
    for c in loads[:3]:
        c.start()

    def perm_rows(val):
        nt = -(-D // 128)
        val = jnp.concatenate([val, jnp.zeros((D, nt * 128 - D), F32)], axis=1)
        for j in range(nt):
            tmp[j * D:(j + 1) * D, :] = val[:, j * 128:(j + 1) * 128]
        return jnp.concatenate([
            jnp.concatenate([tmp[pl.ds(j * D + d, H, stride=DH), :]
                             for d in range(DH)], axis=0)
            for j in range(nt)], axis=1)[:, :D]

    for c in loads[:3]:
        c.wait()
    for c in loads[3:]:
        c.start()
    for p in range(3):
        wq_p[p * D:(p + 1) * D, :] = perm_rows(
            wqkv_v[:, p * D:(p + 1) * D].astype(F32).T).astype(BF)
    wo_p[...] = perm_rows(wo_v[...].astype(F32)).T.astype(BF)
    xs[...] = xin[...].astype(F32)

    lane = jax.lax.broadcasted_iota(jnp.int32, (H, 128), 1)
    c2 = DH ** -0.5 * math.log2(math.e)

    def shifted(cur, prev, w):
        if w == 0:
            return cur.astype(F32)
        sh = DIL * w
        if prev is not None:
            cur = jnp.where(lane >= 128 - sh, prev, cur)
        return pltpu.roll(cur, sh, 1).astype(F32)

    def attend(q, k, v, kp, vp, b):
        r = lambda a, d: None if a is None else a[d * H:(d + 1) * H]
        lg = []
        for w in range(W):
            acc = None
            for d in range(DH):
                t = r(q, d) * shifted(r(k, d), r(kp, d), w)
                acc = t if acc is None else acc + t
            acc = acc * c2
            if b is not None and w > 0:
                acc = jnp.where(lane + b * 128 >= DIL * w, acc, -1e9)
            lg.append(acc)
        m = lg[0]
        for a in lg[1:]:
            m = jnp.maximum(m, a)
        e = [jnp.exp2(a - m) for a in lg]
        inv = 1.0 / sum(e[1:], e[0])
        pr = [a * inv for a in e]
        outs = []
        for d in range(DH):
            acc = None
            for w in range(W):
                t = pr[w] * shifted(r(v, d), r(vp, d), w)
                acc = t if acc is None else acc + t
            outs.append(acc.astype(BF))
        return jnp.concatenate(outs, axis=0)

    nb = S // TB
    blk = lambda t: pl.ds(pl.multiple_of((t % nb) * TB, TB), TB)
    out_copy = lambda b: pltpu.make_async_copy(
        xin.at[:, blk(b)], o_hbm.at[:, blk(b)], sems.at[6 + b])

    def stage(ta, tf):
        if ta is not None:
            x = xs[:, blk(ta)]
            kp, vp = kv[0], kv[1]
        if tf is not None:
            a = xn[:, blk(tf)]
            acc = xs[:, blk(tf)]
        if ta is not None:
            qkv = _dot(wq_p[...], _ln(x))
            os = []
            for t in range(TB // 128):
                c = slice(t * 128, (t + 1) * 128)
                q, k, v = (qkv[p * D:(p + 1) * D, c] for p in range(3))
                k, v = k.astype(KVT), v.astype(KVT)
                os.append(attend(q, k, v, kp, vp, ta % nb if t == 0 else None))
                kp, vp = k, v
            kv[0] = kp
            kv[1] = vp
        def ffn(acc, lo, hi):
            for j in range(lo, hi):
                c = slice(j * FC, (j + 1) * FC)
                g = jax.lax.dot_general(wg[:, c], a, TN, preferred_element_type=F32)
                u = jax.lax.dot_general(wu[:, c], a, TN, preferred_element_type=F32)
                acc = acc + _dot(wd[:, c], (g * u).astype(BF))
            return acc
        if tf is not None:
            acc = ffn(acc, 0, 5)
        if ta is not None:
            x = x + _dot(wo_p[...], jnp.concatenate(os, axis=1))
            xs[:, blk(ta)] = x
            xn[:, blk(ta)] = _ln(x)
        if tf is not None:
            acc = ffn(acc, 5, F // FC)
        if tf is not None:
            xs[:, blk(tf)] = acc
            xin[:, blk(tf)] = acc.astype(BF)

            @pl.when(tf >= nb)
            def _():
                out_copy(tf - nb).start()

    kv[...] = jnp.zeros_like(kv)
    jax.lax.fori_loop(0, LA, lambda t, _: stage(t, None), None)
    for c in loads[3:]:
        c.wait()
    jax.lax.fori_loop(0, 2 * nb - LA, lambda t, _: stage(t + LA, t), None)
    jax.lax.fori_loop(2 * nb - LA, 2 * nb, lambda t, _: stage(None, t), None)
    for b in range(nb):
        out_copy(b).wait()


@jax.jit
def pallas_interleave_layers__sliding_local_dilated__glu_gated_bilinear__prompt_kernel(
    A_x: jax.Array,
    A_wqkv: jax.Array,
    A_wo: jax.Array,
    B_x: jax.Array,
    B_w_gate: jax.Array,
    B_w_up: jax.Array,
    B_w_down: jax.Array,
):
    _, S, D = A_x.shape
    F = B_w_gate.shape[1]
    V = pltpu.VMEM
    out = pl.pallas_call(
        _kernel,
        in_specs=[pl.BlockSpec(memory_space=pl.ANY)] * 6,
        out_specs=pl.BlockSpec(memory_space=pl.ANY),
        out_shape=jax.ShapeDtypeStruct((D, S), A_x.dtype),
        scratch_shapes=[
            V((D, S), BF), V((D, 3 * D), BF), V((D, D), BF),
            V((D, F), BF), V((D, F), BF), V((D, F), BF),
            V((3 * D, D), BF), V((D, D), BF), V((-(-D // 128) * D, 128), F32),
            V((D, S), F32), V((D, S), BF), V((2, D, 128), KVT),
            pltpu.SemaphoreType.DMA((6 + S // TB,)),
        ],
        compiler_params=pltpu.CompilerParams(vmem_limit_bytes=100 << 20),
    )(A_x[0].T, A_wqkv, A_wo, B_w_gate, B_w_up, B_w_down.T)
    return out.T[None]
```
